```python
import jax
import jax.numpy as jnp

def _softmax(x, axis=-1):
    return jax.nn.softmax(x, axis=axis)

def _gelu(x):
    return jax.nn.gelu(x, approximate=True)

def _silu(x):
    return jax.nn.silu(x)

def _sigmoid(x):
    return jax.nn.sigmoid(x)

def _layernorm(x, axis=-1, eps=1e-05):
    m = jnp.mean(x, axis=axis, keepdims=True)
    v = jnp.var(x, axis=axis, keepdims=True)
    return (x - m) / jnp.sqrt(v + eps)

def _scatter_add(tgt, idx, src, axis=0):
    return tgt.at[idx].add(src)

def _segment_sum(src, seg, n):
    return jax.ops.segment_sum(src, seg, n)

class _Rng:

    def __init__(self, key):
        self._k = key

    def _next(self):
        self._k, sub = jax.random.split(self._k)
        return sub

    def normal(self, shape):
        return jax.random.normal(self._next(), shape, dtype=jnp.bfloat16)

    def randint(self, lo, hi, shape):
        return jax.random.randint(self._next(), shape, lo, hi, dtype=jnp.int32)

    def uniform(self, shape, lo=0.0, hi=1.0):
        return jax.random.uniform(self._next(), shape, jnp.bfloat16, lo, hi)

    def permutation(self, n):
        return jax.random.permutation(self._next(), n)
kernel_name = 'interleave_layers__linear_kernel_hedgehog__mixer_gmlp__prompt'

def _fwd_setup_inputs():
    _rng = _Rng(jax.random.key(int.from_bytes(__import__("os").urandom(4), "little")))
    _w = lambda a: (lambda t: t.astype(jnp.bfloat16) if jnp.issubdtype(t.dtype, jnp.floating) else t)(jnp.asarray(a))

    def _A_setup():
        B, S, D, H = (1, 2048, 640, 32)
        Dh = D // H
        return {'x': _w((lambda *s: _rng.normal(s) * 0.05)(B, S, D)), 'wqkv': _w((lambda *s: _rng.normal(s) * 0.05)(D, 3 * D)), 'w_phi': _w((lambda *s: _rng.normal(s) * 0.05)(H, Dh, Dh) * Dh ** (-0.5)), 'wo': _w((lambda *s: _rng.normal(s) * 0.05)(D, D))}
    _A_in = _A_setup()

    def _B_setup():
        B, S, D, F = (1, 2048, 640, 1536)
        Fh = F // 2
        return {'x': _w((lambda *s: _rng.normal(s) * 0.05)(B, S, D)), 'w_in': _w((lambda *s: _rng.normal(s) * 0.05)(D, 2 * Fh)), 'w_sp': _w(0.01 * (lambda *s: _rng.normal(s) * 0.05)(S, S)), 'b_sp': _w(1.0 + 0.01 * (lambda *s: _rng.normal(s) * 0.05)(S)), 'w_out': _w((lambda *s: _rng.normal(s) * 0.05)(Fh, D))}
    _B_in = _B_setup()
    return {'A_x': _A_in['x'], 'A_wqkv': _A_in['wqkv'], 'A_w_phi': _A_in['w_phi'], 'A_wo': _A_in['wo'], 'B_x': _B_in['x'], 'B_w_in': _B_in['w_in'], 'B_w_sp': _B_in['w_sp'], 'B_b_sp': _B_in['b_sp'], 'B_w_out': _B_in['w_out']}

def _fwd_reference(A_x, A_wqkv, A_w_phi, A_wo, B_x, B_w_in, B_w_sp, B_b_sp, B_w_out):

    def _A_ref(x, wqkv, w_phi, wo):
        B, S, D = x.shape
        H = 32
        Dh = D // H
        qkv = (lambda x, *d: x.transpose(*d))((x @ wqkv).reshape(B, S, 3, H, Dh), 2, 0, 3, 1, 4)
        q, k, v = (qkv[0], qkv[1], qkv[2])
        pq = jnp.einsum('bhsd,hdf->bhsf', q, w_phi)
        pk = jnp.einsum('bhsd,hdf->bhsf', k, w_phi)
        phi_q = jnp.concatenate([_softmax(pq, axis=-1), _softmax(-pq, axis=-1)], axis=-1)
        phi_k = jnp.concatenate([_softmax(pk, axis=-1), _softmax(-pk, axis=-1)], axis=-1)
        kv = jnp.einsum('bhsf,bhsd->bhfd', phi_k, v)
        z = jnp.einsum('bhsf->bhf', phi_k)
        num = jnp.einsum('bhqf,bhfd->bhqd', phi_q, kv)
        den = jnp.einsum('bhqf,bhf->bhq', phi_q, z)[..., None] + 1e-06
        o = num / den
        return (lambda x, *d: x.transpose(*d))(o, 0, 2, 1, 3).reshape(B, S, D) @ wo

    def _B_ref(x, w_in, w_sp, b_sp, w_out):
        B, S, D = x.shape
        F = w_in.shape[-1]
        Fh = F // 2
        z = _gelu(jnp.einsum('bsd,df->bsf', x, w_in))
        z1 = z[..., :Fh].copy()
        z2 = _layernorm(z[..., Fh:], axis=-1)
        g = jnp.einsum('ts,bsf->btf', w_sp, z2) + b_sp[None, :, None]
        return jnp.einsum('bsf,fd->bsd', z1 * g, w_out)
    x = A_x
    x = x + _A_ref(_layernorm(x, axis=-1), A_wqkv, A_w_phi, A_wo)
    x = x + _B_ref(_layernorm(x, axis=-1), B_w_in, B_w_sp, B_b_sp, B_w_out)
    x = x + _A_ref(_layernorm(x, axis=-1), A_wqkv, A_w_phi, A_wo)
    x = x + _B_ref(_layernorm(x, axis=-1), B_w_in, B_w_sp, B_b_sp, B_w_out)
    return x

def setup_inputs():
    _inp = _fwd_setup_inputs()
    _gk = jax.random.fold_in(jax.random.key(int.from_bytes(__import__("os").urandom(4), "little")), 2 ** 31 - 1)
    _shapes = [[1, 2048, 640]]
    _dtypes = ['bfloat16']
    _gks = jax.random.split(_gk, len(_shapes))
    _gs = [jax.random.normal(k, s, dtype=jnp.dtype(d)) * 0.05 for k, s, d in zip(_gks, _shapes, _dtypes)]
    _inp['grad_out'] = _gs[0]
    return _inp

def reference(A_x, A_wqkv, A_w_phi, A_wo, B_w_in, B_w_sp, B_b_sp, B_w_out, B_x, grad_out):
    _const = dict(B_x=B_x)

    def _f(*_d):
        return _fwd_reference(**{'A_x': _d[0], 'A_wqkv': _d[1], 'A_w_phi': _d[2], 'A_wo': _d[3], 'B_w_in': _d[4], 'B_w_sp': _d[5], 'B_b_sp': _d[6], 'B_w_out': _d[7], **_const})
    _out, _vjp = jax.vjp(_f, A_x, A_wqkv, A_w_phi, A_wo, B_w_in, B_w_sp, B_b_sp, B_w_out)
    _grads = _vjp(grad_out)
    _out0 = jnp.asarray(_out)
    return (_out0, *[jnp.asarray(_g) for _g in _grads])
```

```python
import math

import jax
import jax.numpy as jnp
from jax import lax
import jax.experimental.pallas as pl
import jax.experimental.pallas.tpu as pltpu

S = 2048
D = 640
H = 32
DH = 20
F = 1536
FH = 768
NG = 4
HG = 8
GR = DH * HG
VA = GR + 16
TC = 512
NC = S // TC
MB = 128
EPS = 1e-5
LOG2E = math.log2(math.e)

A_H = 0
A_Q = A_H + D
A_K = A_Q + 2 * D
A_V = A_K + 2 * D
A_O = A_V + NG * VA
A_ROWS = A_O + D
B_H = 0
B_U = B_H + D
B_G = B_U + F
B_ROWS = B_G + FH

BF = jnp.bfloat16
F32 = jnp.float32
U32 = jnp.uint32
ALL = slice(None)

_NN = (((1,), (0,)), ((), ()))
_NT = (((1,), (1,)), ((), ()))
_TN = (((0,), (0,)), ((), ()))


def _mm(a, b, dims=_NN):
    return lax.dot_general(a, b, dims, preferred_element_type=F32)


def _csum(x):
    return jnp.sum(x, axis=0, keepdims=True)


def _ld(ref, r0, r1, cs=ALL, lead=()):
    return pltpu.bitcast(ref[(*lead, slice(r0 // 2, r1 // 2), cs)], BF)


def _st(ref, r0, r1, cs, v, lead=()):
    ref[(*lead, slice(r0 // 2, r1 // 2), cs)] = pltpu.bitcast(v.astype(BF), U32)


def _pk(shape):
    return pltpu.VMEM((*shape[:-2], shape[-2] // 2, shape[-1]), U32)


_GC = math.sqrt(2.0 / math.pi)


def _gelu(u):
    t = jnp.tanh(_GC * (u + 0.044715 * (u * u * u)))
    return 0.5 * u * (1.0 + t)


def _gelu_and_grad(u):
    u2 = u * u
    t = jnp.tanh(_GC * (u + 0.044715 * (u2 * u)))
    hp = 0.5 * (1.0 + t)
    z = u * hp
    dz = hp + (0.5 * _GC) * u * (1.0 - t * t) * (1.0 + (3.0 * 0.044715) * u2)
    return z, dz


def _kv_mask():
    r = lax.broadcasted_iota(jnp.int32, (VA, 2 * GR), 0)
    c = lax.broadcasted_iota(jnp.int32, (VA, 2 * GR), 1)
    return jnp.logical_and((r & 7) == (c & 7), r < GR + HG)


def _blocks(n):
    return [(m, min(m + MB, n)) for m in range(0, n, MB)]


def _acc(total, t):
    return t if total is None else total + t


def _kernel(
    x_hbm, wqkv_hbm, wphi_hbm, wo_hbm, win_hbm, wsp_hbm, bsp_hbm, wout_hbm, g_hbm,
    out_hbm, gx_hbm, dwqkv_hbm, dwphi_hbm, dwo_hbm, dwin_hbm, dwsp_hbm, dbsp_hbm,
    dwout_hbm, spill_hbm,
    xs, ra, rb, z2c, stats, invden, kvm, kvmt,
    wqkvt, wp, wop, win, wout, wsp, bsp, mg, pg, outst, gin, stg, stb,
    dxs, acc_wp, acc_wop, acc_win, acc_wout, acc_bsp, sems,
):
    def cp(src, dst, k):
        return pltpu.make_async_copy(src, dst, sems.at[k])

    def chunk(c):
        return pl.ds(pl.multiple_of(c * TC, TC), TC)

    def loop(name, body):
        with jax.named_scope(name):
            lax.fori_loop(0, NC, body, 0, unroll=1)

    def ln_fwd(src, n, src_cs, dst, d0, cs, stat_row):
        s1 = None
        for a, b in _blocks(n):
            s1 = _acc(s1, _csum(src[a:b, src_cs]))
        mu = s1 * (1.0 / n)
        s2 = None
        for a, b in _blocks(n):
            xc = src[a:b, src_cs] - mu
            s2 = _acc(s2, _csum(xc * xc))
        rstd = lax.rsqrt(s2 * (1.0 / n) + EPS)
        stats[stat_row:stat_row + 1, cs] = rstd
        for a, b in _blocks(n):
            _st(dst, d0 + a, d0 + b, cs, (src[a:b, src_cs] - mu) * rstd)

    spill_rows_a = slice(0, A_ROWS // 2)
    spill_rows_b = slice(A_ROWS // 2, (A_ROWS + B_ROWS) // 2)

    def fwd_scope(xin, wo_raw, wqkv, wphi, win_raw, wout_raw, stw,
                  wpt, wopt, wint, woutt):
        in_copies = [
            cp(x_hbm, xin, 0), cp(wqkv_hbm, wqkv, 1), cp(wphi_hbm, wphi, 2),
            cp(wo_hbm, wo_raw, 3), cp(win_hbm, win_raw, 4), cp(bsp_hbm, bsp, 5),
            cp(wout_hbm, wout_raw, 6), cp(wsp_hbm, wsp, 7), cp(g_hbm, gin, 8),
        ]
        for c in in_copies:
            c.start()

        o_col = lax.broadcasted_iota(jnp.int32, (1, GR), 1)
        r_row = lax.broadcasted_iota(jnp.int32, (GR, 1), 0)
        ho_col = o_col // DH
        same = ho_col == (r_row & 7)
        _st(pg, 0, GR, ALL, jnp.where(
            jnp.logical_and(same, o_col - ho_col * DH == (r_row >> 3)), 1.0, 0.0))
        fe = lax.broadcasted_iota(jnp.int32, (1, 128), 1)
        er = jnp.where(fe == (r_row >> 3), 1.0, 0.0).astype(BF)

        in_copies[0].wait()

        def load_x(c, carry):
            rows = chunk(c)
            xs[:, rows] = xin[rows, :].astype(F32).T
            return carry
        loop('load_x', load_x)

        in_copies[2].wait()
        for g in range(NG):
            t = _mm(er, wphi[GR * g:GR * (g + 1), :], _NT)
            _st(mg, 0, GR, ALL, jnp.where(same, t, 0.0), lead=(g,))

        in_copies[1].wait()
        for i in range(3):
            _st(wqkvt, i * D, (i + 1) * D, ALL, wqkv[:, i * D:(i + 1) * D].astype(F32).T)
        for i in range(3):
            for g in range(NG):
                r0 = i * D + GR * g
                m = _ld(pg, 0, GR) if i == 2 else _ld(mg, 0, GR, lead=(g,))
                w = _mm(m, _ld(wqkvt, r0, r0 + GR))
                stw[GR * g:GR * (g + 1), :] = w
                if i < 2:
                    w = w * LOG2E
                _st(wpt, r0, r0 + GR, ALL, w)
            _st(wp, 0, D, slice(i * D, (i + 1) * D), stw[...].T)

        in_copies[3].wait()
        for g in range(NG):
            stw[GR * g:GR * (g + 1), :] = _mm(_ld(pg, 0, GR), wo_raw[GR * g:GR * (g + 1), :])
        _st(wop, 0, D, ALL, stw[...])
        _st(wopt, 0, D, ALL, stw[...].T)

        mask = _kv_mask()

        def a_fwd(l):
            def p1(c, carry):
                cs = chunk(c)
                ln_fwd(xs, D, cs, ra, A_H, cs, 2 * l)
                hb = _ld(ra, A_H, A_H + D, cs)
                for base, off in ((A_Q, 0), (A_K, D)):
                    for g in range(NG):
                        o = base + 2 * GR * g
                        pp = _mm(_ld(wpt, off + GR * g, off + GR * (g + 1)), hb)
                        pp = pp.reshape(DH, HG, TC)
                        ep = jnp.exp2(pp - jnp.max(pp, axis=0, keepdims=True))
                        ep = ep * (1.0 / jnp.sum(ep, axis=0, keepdims=True))
                        _st(ra, o, o + GR, cs, ep.reshape(GR, TC))
                        en = jnp.exp2(jnp.min(pp, axis=0, keepdims=True) - pp)
                        en = en * (1.0 / jnp.sum(en, axis=0, keepdims=True))
                        _st(ra, o + GR, o + 2 * GR, cs, en.reshape(GR, TC))
                ones = jnp.ones((VA - GR, TC), BF)
                for g in range(NG):
                    o = A_V + VA * g
                    _st(ra, o, o + GR, cs,
                        _mm(_ld(wpt, 2 * D + GR * g, 2 * D + GR * (g + 1)), hb))
                    _st(ra, o + GR, o + VA, cs, ones)
                return carry
            loop(f'afwd{l}_p1', p1)

            if l == 0:
                in_copies[4].wait()
                in_copies[6].wait()
                _st(win, 0, D, ALL, win_raw[...])
                _st(wout, 0, FH, ALL, wout_raw[...])
                _st(wint, 0, F, ALL, win_raw[...].astype(F32).T)
                _st(woutt, 0, D, ALL, wout_raw[...].astype(F32).T)
            for g in range(NG):
                va = _ld(ra, A_V + VA * g, A_V + VA * (g + 1))
                pk = _ld(ra, A_K + 2 * GR * g, A_K + 2 * GR * (g + 1))
                kv = jnp.where(mask, _mm(va, pk, _NT), 0.0)
                _st(kvm, 0, VA, ALL, kv, lead=(l, g))
                _st(kvmt, 0, 2 * GR, ALL, kv.T, lead=(l, g))

            def p2(c, carry):
                cs = chunk(c)
                for g in range(NG):
                    na = _mm(_ld(kvm, 0, VA, lead=(l, g)),
                             _ld(ra, A_Q + 2 * GR * g, A_Q + 2 * GR * (g + 1), cs))
                    inv = 1.0 / (na[GR:GR + HG] + 1e-6)
                    invden[l, HG * g:HG * (g + 1), cs] = inv
                    o = na[:GR].reshape(DH, HG, TC) * inv[None]
                    _st(ra, A_O + GR * g, A_O + GR * (g + 1), cs, o.reshape(GR, TC))
                xs[:, cs] = xs[:, cs] + _mm(_ld(wopt, 0, D), _ld(ra, A_O, A_O + D, cs))
                return carry
            loop(f'afwd{l}_p2', p2)

        def b_fwd(l):
            def p1(c, carry):
                cs = chunk(c)
                ln_fwd(xs, D, cs, rb, B_H, cs, 2 * l + 1)
                hb = _ld(rb, B_H, B_H + D, cs)
                for a, b in _blocks(F):
                    ub = _mm(_ld(wint, a, b), hb).astype(BF)
                    _st(rb, B_U + a, B_U + b, cs, ub)
                    z = _gelu(ub.astype(F32))
                    if a < FH:
                        _st(rb, B_G + a, B_G + b, cs, z)
                    else:
                        stg[a - FH:b - FH, :] = z
                ln_fwd(stg, FH, ALL, z2c, FH * l, cs, 4 + l)
                return carry
            loop(f'bfwd{l}_p1', p1)

            def p2(c, carry):
                cs = chunk(c)
                wrow = wsp[cs, :]
                bias = bsp[:, cs].astype(F32)
                for a, b in _blocks(FH):
                    gb = (_mm(_ld(z2c, FH * l + a, FH * l + b), wrow, _NT) + bias).astype(BF)
                    z1 = _ld(rb, B_G + a, B_G + b, cs).astype(F32)
                    _st(rb, B_G + a, B_G + b, cs, gb)
                    _st(stb, a, b, ALL, z1 * gb.astype(F32))
                ab = _ld(stb, 0, FH)
                for a, b in _blocks(D):
                    xs[a:b, cs] = xs[a:b, cs] + _mm(_ld(woutt, a, b), ab)
                if l == 1:
                    outst[cs, :] = xs[:, cs].T.astype(BF)
                    dxs[:, cs] = gin[cs, :].astype(F32).T
                    for acc in (acc_wp, acc_wop, acc_win, acc_wout):
                        n = acc.shape[0] // NC
                        acc[pl.ds(pl.multiple_of(c * n, 8), n), :] = jnp.zeros(
                            (n, acc.shape[1]), F32)
                    acc_bsp[:, cs] = jnp.zeros((1, TC), F32)
                return carry
            loop(f'bfwd{l}_p2', p2)

        spill_a = cp(ra, spill_hbm.at[spill_rows_a, :], 9)
        spill_b = cp(rb, spill_hbm.at[spill_rows_b, :], 10)

        a_fwd(0)
        spill_a.start()
        in_copies[5].wait()
        in_copies[7].wait()
        b_fwd(0)
        spill_b.start()
        spill_a.wait()
        a_fwd(1)
        spill_b.wait()
        in_copies[8].wait()
        b_fwd(1)
        cp(outst, out_hbm, 11).start()

    pl.run_scoped(
        fwd_scope,
        pltpu.VMEM((S, D), BF),
        pltpu.VMEM((D, D), BF),
        pltpu.VMEM((D, 3 * D), BF),
        pltpu.VMEM((D, 128), BF),
        pltpu.VMEM((D, F), BF),
        pltpu.VMEM((FH, D), BF),
        pltpu.VMEM((D, D), F32),
        _pk((3 * D, D)),
        _pk((D, D)),
        _pk((F, D)),
        _pk((D, FH)),
    )

    def bwd_scope(acc_kv, dg, dgt, dpq, dkvm, dkvmt,
                  st_wqkv, st_wo, st_win, st_wout, st_wsp, st_wphi, st_bsp, stf):
        mask = _kv_mask()
        reload_b = cp(spill_hbm.at[spill_rows_b, :], rb, 12)
        reload_a = cp(spill_hbm.at[spill_rows_a, :], ra, 13)

        def ln_bwd_into_dxs(cs, h_ref, h0, stat_row):
            s1 = s2 = None
            for a, b in _blocks(D):
                dh = stg[a:b, :]
                s1 = _acc(s1, _csum(dh))
                s2 = _acc(s2, _csum(dh * _ld(h_ref, h0 + a, h0 + b, cs).astype(F32)))
            m1 = s1 * (1.0 / D)
            m2 = s2 * (1.0 / D)
            rstd = stats[stat_row:stat_row + 1, cs]
            for a, b in _blocks(D):
                h = _ld(h_ref, h0 + a, h0 + b, cs).astype(F32)
                dxs[a:b, cs] = dxs[a:b, cs] + rstd * (stg[a:b, :] - m1 - h * m2)

        def b_bwd(l):
            def p1(c, carry):
                cs = chunk(c)
                crow = pl.ds(pl.multiple_of(c * (TC // 2), TC // 2), TC // 2)
                dyb = dxs[:, cs].astype(BF)
                sb = None
                for a, b in _blocks(FH):
                    da = _mm(_ld(wout, a, b), dyb)
                    z1, gp1 = _gelu_and_grad(_ld(rb, B_U + a, B_U + b, cs).astype(F32))
                    g = _ld(rb, B_G + a, B_G + b, cs).astype(F32)
                    acc_wout[a:b, :] += _mm((z1 * g).astype(BF), dyb, _NT)
                    _st(rb, B_U + a, B_U + b, cs, da * g * gp1)
                    dgc = da * z1
                    sb = _acc(sb, _csum(dgc))
                    _st(dg, a, b, cs, dgc)
                    dgt[crow, FH * l + a:FH * l + b] = pltpu.bitcast(dgc.T.astype(BF), U32)
                acc_bsp[:, cs] += sb
                return carry
            loop(f'bbwd{l}_p1', p1)

            def p2(c, carry):
                cs = chunk(c)
                wcol = wsp[:, cs]
                hb = _ld(rb, B_H, B_H + D, cs)
                du1 = _ld(rb, B_U, B_U + FH, cs)
                s1 = s2 = None
                for a, b in _blocks(FH):
                    dz2 = _mm(_ld(dg, a, b), wcol)
                    stg[a:b, :] = dz2
                    s1 = _acc(s1, _csum(dz2))
                    s2 = _acc(s2, _csum(
                        dz2 * _ld(z2c, FH * l + a, FH * l + b, cs).astype(F32)))
                for a, b in _blocks(D):
                    acc_win[a:b, 0:FH] += _mm(hb[a:b], du1, _NT)
                m1 = s1 * (1.0 / FH)
                m2 = s2 * (1.0 / FH)
                rstd2 = stats[4 + l:5 + l, cs]
                for a, b in _blocks(FH):
                    z2 = _ld(z2c, FH * l + a, FH * l + b, cs).astype(F32)
                    dzz = rstd2 * (stg[a:b, :] - m1 - z2 * m2)
                    _, gp2 = _gelu_and_grad(
                        _ld(rb, B_U + FH + a, B_U + FH + b, cs).astype(F32))
                    _st(rb, B_U + FH + a, B_U + FH + b, cs, dzz * gp2)
                du = _ld(rb, B_U, B_U + F, cs)
                for a, b in _blocks(D):
                    stg[a:b, :] = _mm(_ld(win, a, b), du)
                for a, b in _blocks(D):
                    acc_win[a:b, FH:F] += _mm(hb[a:b], du[FH:F], _NT)
                ln_bwd_into_dxs(cs, rb, B_H, 2 * l + 1)
                return carry
            loop(f'bbwd{l}_p2', p2)

        def softmax_bwd(ph, dph):
            php = ph[:GR].reshape(DH, HG, TC)
            phn = ph[GR:].reshape(DH, HG, TC)
            dp_ = dph[:GR].reshape(DH, HG, TC)
            dn_ = dph[GR:].reshape(DH, HG, TC)
            a = php * (dp_ - jnp.sum(php * dp_, axis=0, keepdims=True))
            b = phn * (dn_ - jnp.sum(phn * dn_, axis=0, keepdims=True))
            return (a - b).reshape(GR, TC)

        def a_bwd(l):
            acc_kv[...] = jnp.zeros(acc_kv.shape, F32)

            def p1(c, carry):
                cs = chunk(c)
                dyb = dxs[:, cs].astype(BF)
                do = _mm(_ld(wop, 0, D), dyb)
                ob = _ld(ra, A_O, A_O + D, cs)
                acc_wop[...] += _mm(ob, dyb, _NT)
                of = ob.astype(F32)
                for g in range(NG):
                    dog = do[GR * g:GR * (g + 1)].reshape(DH, HG, TC)
                    og = of[GR * g:GR * (g + 1)].reshape(DH, HG, TC)
                    inv = invden[l, HG * g:HG * (g + 1), cs]
                    dnum = (dog * inv[None]).reshape(GR, TC)
                    dden = -jnp.sum(dog * og, axis=0) * inv
                    dna = jnp.concatenate(
                        [dnum, dden, jnp.zeros((HG, TC), F32)], axis=0).astype(BF)
                    phq = _ld(ra, A_Q + 2 * GR * g, A_Q + 2 * GR * (g + 1), cs)
                    acc_kv[g] += _mm(dna, phq, _NT)
                    dphq = _mm(_ld(kvmt, 0, 2 * GR, lead=(l, g)), dna)
                    _st(dpq, GR * g, GR * (g + 1), cs, softmax_bwd(phq.astype(F32), dphq))
                return carry
            loop(f'abwd{l}_p1', p1)

            for g in range(NG):
                dk = jnp.where(mask, acc_kv[g], 0.0)
                _st(dkvm, 0, VA, ALL, dk, lead=(g,))
                _st(dkvmt, 0, 2 * GR, ALL, dk.T, lead=(g,))

            def p2(c, carry):
                cs = chunk(c)
                hb = _ld(ra, A_H, A_H + D, cs)
                dq = _ld(dpq, 0, D, cs)
                stb[0:D // 2, :] = dpq[:, cs]
                for g in range(NG):
                    va = _ld(ra, A_V + VA * g, A_V + VA * (g + 1), cs)
                    phk = _ld(ra, A_K + 2 * GR * g, A_K + 2 * GR * (g + 1), cs)
                    dphk = _mm(_ld(dkvmt, 0, 2 * GR, lead=(g,)), va)
                    dv = _mm(_ld(dkvm, 0, GR, lead=(g,)), phk)
                    _st(stb, D + GR * g, D + GR * (g + 1), ALL,
                        softmax_bwd(phk.astype(F32), dphk))
                    _st(stb, 2 * D + GR * g, 2 * D + GR * (g + 1), ALL, dv)
                for a, b in _blocks(D):
                    acc_wp[a:b, :] += _mm(dq[a:b], hb, _NT)
                dp = _ld(stb, 0, 3 * D)
                for a, b in _blocks(D):
                    stg[a:b, :] = _mm(_ld(wp, a, b), dp)
                for a, b in _blocks(2 * D):
                    acc_wp[D + a:D + b, :] += _mm(dp[D + a:D + b], hb, _NT)
                ln_bwd_into_dxs(cs, ra, A_H, 2 * l)
                if l == 0:
                    gin[cs, :] = dxs[:, cs].T.astype(BF)
                return carry
            loop(f'abwd{l}_p2', p2)

        b_bwd(1)
        reload_b.start()
        a_bwd(1)
        reload_a.start()
        reload_b.wait()
        b_bwd(0)

        st_win[...] = acc_win[...].astype(BF)
        cp(st_win, dwin_hbm, 14).start()
        st_wout[...] = acc_wout[...].astype(BF)
        cp(st_wout, dwout_hbm, 15).start()
        st_bsp[...] = acc_bsp[...].astype(BF)
        cp(st_bsp, dbsp_hbm, 16).start()

        def wsp_copy(i, slot):
            return cp(st_wsp.at[slot], dwsp_hbm.at[pl.ds(i * TC, TC), :], 17 + slot)

        with jax.named_scope('dwsp'):
            for i in range(NC):
                slot = i % 2
                if i >= 2:
                    wsp_copy(i - 2, slot).wait()
                st_wsp[slot] = _mm(_ld(dgt, i * TC, (i + 1) * TC),
                                   _ld(z2c, 0, 2 * FH)).astype(BF)
                wsp_copy(i, slot).start()

        reload_a.wait()
        a_bwd(0)
        cp(gin, gx_hbm, 19).start()

        o_row = lax.broadcasted_iota(jnp.int32, (GR, 1), 0)
        r_col = lax.broadcasted_iota(jnp.int32, (1, GR), 1)
        same_t = (o_row // DH) == (r_col & 7)
        fe = lax.broadcasted_iota(jnp.int32, (128, 1), 0)
        ef = jnp.where(fe == (r_col >> 3), 1.0, 0.0).astype(BF)

        def wqkv_copy(i):
            return cp(st_wqkv.at[:, i * D:(i + 1) * D], dwqkv_hbm.at[:, i * D:(i + 1) * D],
                      (20, 23, 24)[i])

        for i in range(3):
            for g in range(NG):
                rows = slice(i * D + GR * g, i * D + GR * (g + 1))
                m = _ld(pg, 0, GR) if i == 2 else _ld(mg, 0, GR, lead=(g,))
                stf[GR * g:GR * (g + 1), :] = _mm(m, acc_wp[rows, :].astype(BF), _TN)
            st_wqkv[:, i * D:(i + 1) * D] = stf[...].T.astype(BF)
            wqkv_copy(i).start()
        for g in range(NG):
            rows = slice(GR * g, GR * (g + 1))
            st_wo[rows, :] = _mm(_ld(pg, 0, GR), acc_wop[rows, :].astype(BF), _TN).astype(BF)
        cp(st_wo, dwo_hbm, 21).start()
        for g in range(NG):
            dm = None
            for i in range(2):
                r0 = i * D + GR * g
                dm = _acc(dm, _mm(_ld(wqkvt, r0, r0 + GR),
                                  acc_wp[r0:r0 + GR, :].astype(BF), _NT))
            dm = jnp.where(same_t, dm, 0.0).astype(BF)
            st_wphi[GR * g:GR * (g + 1), :] = _mm(dm, ef, _NT).astype(BF)
        cp(st_wphi, dwphi_hbm, 22).start()

        cp(outst, out_hbm, 11).wait()
        cp(st_win, dwin_hbm, 14).wait()
        cp(st_wout, dwout_hbm, 15).wait()
        cp(st_bsp, dbsp_hbm, 16).wait()
        wsp_copy(NC - 2, 0).wait()
        wsp_copy(NC - 1, 1).wait()
        cp(gin, gx_hbm, 19).wait()
        for i in range(3):
            wqkv_copy(i).wait()
        cp(st_wo, dwo_hbm, 21).wait()
        cp(st_wphi, dwphi_hbm, 22).wait()

    pl.run_scoped(
        bwd_scope,
        pltpu.VMEM((NG, VA, 2 * GR), F32),
        _pk((FH, S)),
        _pk((S, 2 * FH)),
        _pk((D, S)),
        _pk((NG, VA, 2 * GR)),
        _pk((NG, 2 * GR, VA)),
        pltpu.VMEM((D, 3 * D), BF),
        pltpu.VMEM((D, D), BF),
        pltpu.VMEM((D, F), BF),
        pltpu.VMEM((FH, D), BF),
        pltpu.VMEM((2, TC, S), BF),
        pltpu.VMEM((D, 128), BF),
        pltpu.VMEM((1, S), BF),
        pltpu.VMEM((D, D), F32),
    )


@jax.jit
def pallas_interleave_layers__linear_kernel_hedgehog__mixer_gmlp__prompt_kernel(
    A_x: jax.Array,
    A_wqkv: jax.Array,
    A_w_phi: jax.Array,
    A_wo: jax.Array,
    B_x: jax.Array,
    B_w_in: jax.Array,
    B_w_sp: jax.Array,
    B_b_sp: jax.Array,
    B_w_out: jax.Array,
    grad_out: jax.Array,
):
    del B_x
    x2 = A_x.reshape(S, D)
    g2 = grad_out.reshape(S, D)
    wphi2 = jnp.pad(A_w_phi.reshape(D, DH), ((0, 0), (0, 128 - DH)))
    bsp2 = B_b_sp.reshape(1, S)

    any_spec = pl.BlockSpec(memory_space=pl.ANY)
    out_shape = (
        jax.ShapeDtypeStruct((S, D), BF),
        jax.ShapeDtypeStruct((S, D), BF),
        jax.ShapeDtypeStruct((D, 3 * D), BF),
        jax.ShapeDtypeStruct((D, 128), BF),
        jax.ShapeDtypeStruct((D, D), BF),
        jax.ShapeDtypeStruct((D, F), BF),
        jax.ShapeDtypeStruct((S, S), BF),
        jax.ShapeDtypeStruct((1, S), BF),
        jax.ShapeDtypeStruct((FH, D), BF),
        jax.ShapeDtypeStruct(((A_ROWS + B_ROWS) // 2, S), U32),
    )
    scratch = [
        pltpu.VMEM((D, S), F32),
        _pk((A_ROWS, S)),
        _pk((B_ROWS, S)),
        _pk((2 * FH, S)),
        pltpu.VMEM((8, S), F32),
        pltpu.VMEM((2, H, S), F32),
        _pk((2, NG, VA, 2 * GR)),
        _pk((2, NG, 2 * GR, VA)),
        _pk((3 * D, D)),
        _pk((D, 3 * D)),
        _pk((D, D)),
        _pk((D, F)),
        _pk((FH, D)),
        pltpu.VMEM((S, S), BF),
        pltpu.VMEM((1, S), BF),
        _pk((NG, GR, GR)),
        _pk((GR, GR)),
        pltpu.VMEM((S, D), BF),
        pltpu.VMEM((S, D), BF),
        pltpu.VMEM((FH, TC), F32),
        _pk((3 * D, TC)),
        pltpu.VMEM((D, S), F32),
        pltpu.VMEM((3 * D, D), F32),
        pltpu.VMEM((D, D), F32),
        pltpu.VMEM((D, F), F32),
        pltpu.VMEM((FH, D), F32),
        pltpu.VMEM((1, S), F32),
        pltpu.SemaphoreType.DMA((25,)),
    ]
    res = pl.pallas_call(
        _kernel,
        out_shape=out_shape,
        in_specs=[any_spec] * 9,
        out_specs=tuple([any_spec] * 10),
        scratch_shapes=scratch,
        compiler_params=pltpu.CompilerParams(vmem_limit_bytes=127 * 1024 * 1024),
    )(x2, A_wqkv, wphi2, A_wo, B_w_in, B_w_sp, bsp2, B_w_out, g2)
    out, gx, dwqkv, dwphi, dwo, dwin, dwsp, dbsp, dwout, _ = res
    return (
        out.reshape(1, S, D),
        gx.reshape(1, S, D),
        dwqkv,
        dwphi[:, :DH].reshape(H, DH, DH),
        dwo,
        dwin,
        dwsp,
        dbsp.reshape(S),
        dwout,
    )
```
